```python
import jax
import jax.numpy as jnp

def _softmax(x, axis=-1):
    return jax.nn.softmax(x, axis=axis)
def _gelu(x):
    return jax.nn.gelu(x, approximate=True)
def _silu(x):
    return jax.nn.silu(x)
def _sigmoid(x):
    return jax.nn.sigmoid(x)
def _layernorm(x, axis=-1, eps=1e-5):
    m = jnp.mean(x, axis=axis, keepdims=True)
    v = jnp.var(x, axis=axis, keepdims=True)
    return (x - m) / jnp.sqrt(v + eps)
def _scatter_add(tgt, idx, src, axis=0):
    return tgt.at[idx].add(src)
def _segment_sum(src, seg, n):
    return jax.ops.segment_sum(src, seg, n)
class _Rng:
    def __init__(self, key):
        self._k = key
    def _next(self):
        self._k, sub = jax.random.split(self._k)
        return sub
    def normal(self, shape):
        return jax.random.normal(self._next(), shape, dtype=jnp.bfloat16)
    def randint(self, lo, hi, shape):
        return jax.random.randint(self._next(), shape, lo, hi, dtype=jnp.int32)
    def uniform(self, shape, lo=0.0, hi=1.0):
        return jax.random.uniform(self._next(), shape, jnp.bfloat16, lo, hi)
    def permutation(self, n):
        return jax.random.permutation(self._next(), n)


kernel_name = 'concat_heads__ssm_conv_h3__linear_attn_block__prompt'

def setup_inputs():
    _rng = _Rng(jax.random.key(int.from_bytes(__import__("os").urandom(4), "little")))
    _w = (lambda a: (lambda t: t.astype(jnp.bfloat16) if jnp.issubdtype(t.dtype, jnp.floating) else t)(jnp.asarray(a)))
    def _A_setup():
        B, S, D = 1, 2048, 1024
        ks = 4
        return {
            "q": _w((lambda *s: _rng.normal(s) * 0.05)(B, S, D)),
            "k": _w((lambda *s: _rng.normal(s) * 0.05)(B, S, D)),
            "v": _w((lambda *s: _rng.normal(s) * 0.05)(B, S, D)),
            "shift_k": _w((lambda *s: _rng.normal(s) * 0.05)(D, ks) * 0.5),
            "ssm_k": _w((lambda *s: _rng.normal(s) * 0.05)(D, S) * (1.0 / S ** 0.5)),
            "ssm_D": _w((lambda *s: _rng.normal(s) * 0.05)(D)),
        }
    _A_in = _A_setup()

    def _B_setup():
        B, S, D = 1, 2048, 1024
        return {
            "x": _w((lambda *s: _rng.normal(s) * 0.05)(B, S, D)),
            "wqkv": _w((lambda *s: _rng.normal(s) * 0.05)(D, 3 * D)),
            "wo": _w((lambda *s: _rng.normal(s) * 0.05)(D, D)),
        }
    _B_in = _B_setup()

    return {
        "A_q": _A_in["q"],
        "A_k": _A_in["k"],
        "A_v": _A_in["v"],
        "A_shift_k": _A_in["shift_k"],
        "A_ssm_k": _A_in["ssm_k"],
        "A_ssm_D": _A_in["ssm_D"],
        "B_x": _B_in["x"],
        "B_wqkv": _B_in["wqkv"],
        "B_wo": _B_in["wo"],
    }

def reference(A_q, A_k, A_v, A_shift_k, A_ssm_k, A_ssm_D, B_x, B_wqkv, B_wo):
    def _A_ref(q, k, v, shift_k, ssm_k, ssm_D):
        B, S, D = q.shape
        ks = shift_k.shape[-1]
        k_pad = jnp.pad(k, ((0, 0), (ks - 1, 0), (0, 0)))
        k_shift = jnp.zeros_like(k)
        for t in range(ks):
            k_shift = k_shift + k_pad[:, t:t + S, :] * shift_k[:, ks - 1 - t][None, None, :]
        kv = k_shift * v
        L = 2 * S
        kv_pad = jnp.pad(kv, ((0, 0), (0, S), (0, 0)))
        kf_pad = jnp.pad(ssm_k, ((0, 0), (0, S)))
        kv_f = (lambda x, axes=(-2,-1): jnp.fft.rfft2(x.astype(jnp.float32), axes=axes))(kv_pad[:, None, :, :], axes=(1, 2))
        kf_f = (lambda x, axes=(-2,-1): jnp.fft.rfft2(x.astype(jnp.float32), axes=axes))(kf_pad[:, None, :], axes=(1, 2))
        kf_f = (lambda x, *d: x.transpose(*d))(kf_f, 1, 2, 0)
        y_f = kv_f * kf_f[None, :, :, :]
        y = (lambda x, s, axes=(-2,-1): jnp.fft.irfft2(x, s=s, axes=axes).astype(jnp.bfloat16))(y_f, (1, L), axes=(1, 2))[:, 0, :S, :]
        y = y + kv * ssm_D[None, None, :]
        return q * y

    def _B_ref(x, wqkv, wo):
        B, S, D = x.shape
        H = 32; Dh = D // H
        qkv = (lambda x, *d: x.transpose(*d))((x @ wqkv).reshape(B, S, 3, H, Dh), 2, 0, 3, 1, 4)
        q, k, v = qkv[0], qkv[1], qkv[2]
        phi = lambda t: jnp.where(t > 0, t + 1, jnp.exp(t)) + 1e-6
        pq, pk = phi(q), phi(k)
        kv = jnp.einsum("bhsd,bhse->bhde", pk, v)
        z = jnp.einsum("bhsd->bhd", pk)
        num = jnp.einsum("bhqd,bhde->bhqe", pq, kv)
        den = jnp.einsum("bhqd,bhd->bhq", pq, z)[..., None] + 1e-6
        o = num / den
        return (lambda x, *d: x.transpose(*d))(o, 0, 2, 1, 3).reshape(B, S, D) @ wo

    a = _A_ref(A_q, A_k, A_v, A_shift_k, A_ssm_k, A_ssm_D)
    b = _B_ref(B_x, B_wqkv, B_wo)
    return jnp.concatenate([a, b], axis=-1)
```

```python
import jax
import jax.numpy as jnp
import numpy as np
import ml_dtypes
import jax.experimental.pallas as pl
import jax.experimental.pallas.tpu as pltpu

S, D, P, NB, NT = 2048, 1024, 128, 16, 8
f32, bf16 = jnp.float32, jnp.bfloat16

_th = np.pi * (2 * np.arange(P)[:, None] + 1) * np.arange(P)[None, :] / (2 * P)
_F = np.concatenate([np.cos(_th), -np.sin(_th)], 0).astype(ml_dtypes.bfloat16)
_G = (np.concatenate([np.cos(_th).T, -np.sin(_th).T], 1) / P).astype(ml_dtypes.bfloat16)


def _dot(a, b, dims=((1,), (0,))):
    return jax.lax.dot_general(a, b, (dims, ((), ())), preferred_element_type=f32)


def _kernel(q_h, k_h, v_h, sk_ref, h_h, d_ref, x_h, w_h, wo_h, f_ref, g_ref, out_h,
            xs, wb, wos, qb, kb, vb, hb, rs, kvw, xre, xim, hre, him, ys, kvf, oa, ob,
            skt, sx, sw, swo, sa, soa, sob):
    def a_copies(t):
        c = pl.ds(t * P, P)
        return [pltpu.make_async_copy(k_h.at[:, c], kb.at[t], sa.at[t, 0]),
                pltpu.make_async_copy(v_h.at[:, c], vb.at[t], sa.at[t, 1]),
                pltpu.make_async_copy(h_h.at[c, :], hb.at[t], sa.at[t, 2]),
                pltpu.make_async_copy(q_h.at[:, c], qb.at[t], sa.at[t, 3])]

    def w_copies(t):
        return [pltpu.make_async_copy(w_h.at[:, pl.ds(j * D + t * P, P)],
                                      wb.at[t, :, pl.ds(j * P, P)], sw.at[t, j]) for j in range(3)]

    XC = 8
    xr = S // XC
    x_copies = [pltpu.make_async_copy(x_h.at[pl.ds(i * xr, xr)], xs.at[pl.ds(i * xr, xr)], sx.at[i])
                for i in range(XC)]
    wo_copy = pltpu.make_async_copy(wo_h, wos, swo)
    oa_copy = lambda t: pltpu.make_async_copy(oa.at[t], out_h.at[:, pl.ds(t * P, P)], soa.at[t])
    ob_copy = lambda i: pltpu.make_async_copy(ob.at[pl.ds(i * xr, xr)],
                                              out_h.at[pl.ds(i * xr, xr), pl.ds(D, D)], sob.at[i])

    for c in a_copies(0)[:3] + w_copies(0) + x_copies + a_copies(0)[3:] + [wo_copy]:
        c.start()

    sk = jnp.concatenate([sk_ref[...].astype(f32), jnp.zeros((D, P - 4), f32)], axis=1)
    skt[...] = sk.T
    dvec = d_ref[...].astype(f32)[None, :]

    row = jax.lax.broadcasted_iota(jnp.int32, (P, P), 0)
    col = jax.lax.broadcasted_iota(jnp.int32, (P, P), 1)
    bd = (row // 32) == (col // 32)
    sgn = jnp.where(jax.lax.broadcasted_iota(jnp.int32, (P, P), 0) % 2 == 0, 1.0, -1.0).astype(f32)

    def phi(t):
        return jnp.where(t > 0, t + 1, jnp.exp(t)) + 1e-6

    for t in range(NT):
        if t + 1 < NT:
            for c in w_copies(t + 1) + a_copies(t + 1):
                c.start()
        cs = slice(t * P, (t + 1) * P)
        ac = a_copies(t)
        ac[0].wait(); ac[1].wait(); ac[2].wait()
        kf = kb[t].astype(f32)
        rid = jax.lax.broadcasted_iota(jnp.int32, (S, P), 0)
        ks = kf * skt[0:1, cs]
        for u in range(1, 4):
            ks = ks + jnp.where(rid >= u, pltpu.roll(kf, u, 0), 0.0) * skt[u:u + 1, cs]
        kv = ks * vb[t].astype(f32)
        kvf[...] = kv
        kvb = kv.astype(bf16)
        fm = f_ref[...]
        for j in range(NB):
            r = slice(j * P, (j + 1) * P)
            X = _dot(fm, kvb[r])
            xre[r] = X[:P]; xim[r] = X[P:]
        prev = None
        for j in range(NB):
            r = slice(j * P, (j + 1) * P)
            H = _dot(fm, hb[t, :, r], ((1,), (1,)))
            a, b = H[:P], H[P:]
            if prev is not None:
                hre[r] = a - sgn * prev[1]; him[r] = b + sgn * prev[0]
            else:
                hre[r] = a; him[r] = b
            prev = (a, b)
        for c in w_copies(t):
            c.wait()
        if t == 0:
            for c in x_copies:
                c.wait()
        qkv = _dot(xs[...], wb[t])
        pq = phi(qkv[:, :P]); pk = phi(qkv[:, P:2 * P]); vv = qkv[:, 2 * P:]
        z = jnp.sum(pk, axis=0, keepdims=True)
        kvm = _dot(pk.astype(bf16).T, vv.astype(bf16))
        kvm = jnp.where(bd, kvm, 0.0).astype(bf16)
        if t == 0:
            wo_copy.wait()
        kvw[cs, :] = _dot(kvm, wos[cs, :]).astype(bf16)
        pqb = pq.astype(bf16)
        zt = jnp.broadcast_to(z, (P, P)).T
        den = _dot(pqb, jnp.where(bd, zt, 0.0).astype(bf16)) + 1e-6
        rs[t] = (pqb.astype(f32) / den).astype(bf16)
        for sl in range(P // 8):
            for ib in range(0, NB, 4):
                acc = [[None, None] for _ in range(4)]
                for j in range(ib + 4):
                    rj = slice(j * P + sl * 8, j * P + sl * 8 + 8)
                    a, b = xre[rj], xim[rj]
                    for ii in range(4):
                        m = ib + ii - j
                        if m < 0:
                            continue
                        rm = slice(m * P + sl * 8, m * P + sl * 8 + 8)
                        c, d = hre[rm], him[rm]
                        pr, pi = a * c - b * d, a * d + b * c
                        if acc[ii][0] is None:
                            acc[ii] = [pr, pi]
                        else:
                            acc[ii] = [acc[ii][0] + pr, acc[ii][1] + pi]
                for ii in range(4):
                    xre_i = ib + ii
                    ys[xre_i, sl * 8:sl * 8 + 8, :] = acc[ii][0]
                    ys[xre_i, P + sl * 8:P + sl * 8 + 8, :] = acc[ii][1]
        ac[3].wait()
        gm = g_ref[...]
        for i in range(NB):
            r = slice(i * P, (i + 1) * P)
            y = _dot(gm, ys[i].astype(bf16))
            oa[t, r, :] = (qb[t, r, :].astype(f32) * (y + kvf[r] * dvec[:, cs])).astype(bf16)
        oa_copy(t).start()

    for i in range(XC):
        r = slice(i * xr, (i + 1) * xr)
        rr = jnp.concatenate([rs[g, r, :] for g in range(NT)], axis=1)
        ob[r] = _dot(rr, kvw[...]).astype(bf16)
        ob_copy(i).start()
    for t in range(NT):
        oa_copy(t).wait()
    for i in range(XC):
        ob_copy(i).wait()


@jax.jit
def pallas_concat_heads__ssm_conv_h3__linear_attn_block__prompt_kernel(
    A_q, A_k, A_v, A_shift_k, A_ssm_k, A_ssm_D, B_x, B_wqkv, B_wo):
    hbm = pl.BlockSpec(memory_space=pl.ANY)
    vm = pl.BlockSpec(memory_space=pltpu.VMEM)
    V = pltpu.VMEM
    DMA = pltpu.SemaphoreType.DMA
    out = pl.pallas_call(
        _kernel,
        out_shape=jax.ShapeDtypeStruct((S, 2 * D), bf16),
        in_specs=[hbm, hbm, hbm, vm, hbm, vm, hbm, hbm, hbm, vm, vm],
        out_specs=hbm,
        scratch_shapes=[
            V((S, D), bf16), V((NT, D, 3 * P), bf16), V((D, D), bf16),
            V((NT, S, P), bf16), V((NT, S, P), bf16), V((NT, S, P), bf16), V((NT, P, S), bf16),
            V((NT, S, P), bf16), V((D, D), bf16),
            V((S, P), f32), V((S, P), f32), V((S, P), f32), V((S, P), f32),
            V((NB, 2 * P, P), f32), V((S, P), f32), V((NT, S, P), bf16), V((S, D), bf16),
            V((P, D), f32),
            DMA((8,)), DMA((NT, 3)), DMA(()), DMA((NT, 4)), DMA((NT,)), DMA((8,)),
        ],
        compiler_params=pltpu.CompilerParams(vmem_limit_bytes=100 * 1024 * 1024),
    )(A_q.reshape(S, D), A_k.reshape(S, D), A_v.reshape(S, D), A_shift_k, A_ssm_k, A_ssm_D,
      B_x.reshape(S, D), B_wqkv, B_wo, _F, _G)
    return out.reshape(1, S, 2 * D)
```

```python
import jax
import jax.numpy as jnp
import numpy as np
import ml_dtypes
import jax.experimental.pallas as pl
import jax.experimental.pallas.tpu as pltpu

S, D, P, NB, NT = 2048, 1024, 128, 16, 8
f32, bf16 = jnp.float32, jnp.bfloat16

_th = np.pi * (2 * np.arange(P)[:, None] + 1) * np.arange(P)[None, :] / (2 * P)
_F = np.concatenate([np.cos(_th), -np.sin(_th)], 0).astype(ml_dtypes.bfloat16)
_G = (np.concatenate([np.cos(_th).T, -np.sin(_th).T], 1) / P).astype(ml_dtypes.bfloat16)


def _dot(a, b, dims=((1,), (0,))):
    return jax.lax.dot_general(a, b, (dims, ((), ())), preferred_element_type=f32)


LOOP = False
NC = 8
KS = 1
OR = S // 8
CR = S // NC


def _kernel(q_h, k_h, v_h, sk_ref, h_h, d_ref, x_h, w_h, wo_h, f_ref, g_ref, z_ref, out_h,
            xs, wb, wos, qb, kb, vb, hb, rs, kvw, xh, ys, kvf, oa, ob,
            taps, kvacc, zacc, flag, sx, sw, swo, sa, soa, sob):
    flag[0] = 0
    dep = [None]

    def setdep(v):
        dep[0] = pltpu.bitcast(v, jnp.int32) & z_ref[...]

    def tie(w):
        if dep[0] is None:
            return w
        parts = []
        for k in range(0, w.shape[0], P):
            st = pltpu.bitcast(pltpu.bitcast(w[k:k + 16], jnp.int32) | dep[0], bf16)
            parts += [st, w[k + 16:k + P]]
        return jnp.concatenate(parts, axis=0)

    def blk(f):
        f()
        if newdep:
            setdep(newdep[-1])
            newdep.clear()

    def cds(t):
        return pl.ds(t * P if isinstance(t, int) else pl.multiple_of(t * P, P), P)

    def a_copy(t, n):
        src, dst = ((k_h, kb), (v_h, vb), (h_h, hb), (q_h, qb))[n]
        src = src.at[cds(t), :] if n == 2 else src.at[:, cds(t)]
        return pltpu.make_async_copy(src, dst.at[t], sa.at[t, n])

    def w_copy(t, j):
        c = pl.ds(j * D + t * P if isinstance(t, int) else pl.multiple_of(j * D + t * P, P), P)
        return pltpu.make_async_copy(w_h.at[:, c], wb.at[t, j], sw.at[t, j])

    class Multi:
        def __init__(self, cs):
            self.cs = cs

        def start(self):
            for c in self.cs:
                c().start()

        def wait(self):
            for c in self.cs:
                c().wait()

    XR = S // 4

    def x_copy(i):
        r = pl.ds(i * XR, XR)
        return Multi([lambda g=g: pltpu.make_async_copy(x_h.at[r, pl.ds(g * P, P)], xs.at[g, r], sx.at[i, g])
                      for g in range(NT)])

    wo_copy = pltpu.make_async_copy(wo_h, wos, swo)

    def oa_copy(t):
        return pltpu.make_async_copy(oa.at[t], out_h.at[:, cds(t)], soa.at[t])

    def ob_copy(i):
        r = pl.ds(i * OR, OR)
        return Multi([lambda g=g: pltpu.make_async_copy(ob.at[g, r], out_h.at[r, pl.ds(D + g * P, P)], sob.at[i, g])
                      for g in range(NT)])

    for j in range(3):
        w_copy(0, j).start()
    x_copy(0).start()
    for n in range(3):
        a_copy(0, n).start()
    for i in range(1, 4):
        x_copy(i).start()
    wo_copy.start()

    skt = sk_ref[...].astype(f32)
    dvec = d_ref[...].astype(f32)[None, :]
    for t in range(NT):
        taps[t, 0:4, :] = skt[:, t * P:(t + 1) * P]
        taps[t, 4:5, :] = dvec[:, t * P:(t + 1) * P]

    def bdmask():
        row = jax.lax.broadcasted_iota(jnp.int32, (P, P), 0)
        col = jax.lax.broadcasted_iota(jnp.int32, (P, P), 1)
        return (row // 32) == (col // 32)

    def phi(t):
        return jnp.where(t > 0, t + 1, jnp.exp(t)) + 1e-6

    def b1(t, c, side):
        r = slice(c * CR, (c + 1) * CR)
        qkv = None
        for g in range(0, NT, KS):
            d_ = _dot(jnp.concatenate([xs[e, r] for e in range(g, g + KS)], axis=1),
                      jnp.concatenate([wb[t, j, g * P:(g + KS) * P] for j in range(3)], axis=1))
            qkv = d_ if qkv is None else qkv + d_
            for _ in range(KS * 8 // NC):
                next(side, None)
        for _ in side:
            pass
        rs[t, r] = phi(qkv[:, :P]).astype(bf16)
        pk = phi(qkv[:, P:2 * P])
        z = pk[0:8]
        for i in range(1, CR // 8):
            z = z + pk[8 * i:8 * i + 8]
        m = _dot(pk.astype(bf16).T, qkv[:, 2 * P:].astype(bf16))
        if c == 0:
            zacc[t] = z; kvacc[t] = m
        else:
            zacc[t] += z; kvacc[t] += m

    def bpost(t, c):
        bd = bdmask()
        if c == 0:
            kvm = jnp.where(bd, kvacc[t], 0.0).astype(bf16)
            kw = _dot(kvm, wos[cds(t), :]).astype(bf16)
            for g in range(NT):
                kvw[g, cds(t), :] = kw[:, g * P:(g + 1) * P]
            z = jnp.sum(zacc[t], axis=0, keepdims=True)
            kvacc[t] = jnp.where(bd, jnp.broadcast_to(z, (P, P)).T, 0.0)
        r = slice(c * CR, (c + 1) * CR)
        pq = rs[t, r]
        den = _dot(pq, tie(kvacc[t].astype(bf16))) + 1e-6
        rs[t, r] = (pq.astype(f32) / den).astype(bf16)

    def fwd(t, p, c):
        lo = c * CR
        if c == 0:
            kk = jnp.concatenate([jnp.zeros((16, P), f32), kb[t, 0:CR].astype(f32)], axis=0)
        else:
            kk = kb[t, lo - 16:lo + CR].astype(f32)
        ks = kk * taps[t, 0:1, :]
        for u in range(1, 4):
            ks = ks + pltpu.roll(kk, u, 0) * taps[t, u:u + 1, :]
        kv = ks[16:] * vb[t, lo:lo + CR].astype(f32)
        kvf[t % 3, lo:lo + CR] = kv * taps[t, 4:5, :]
        kvb = tie(kv.astype(bf16))
        fm = f_ref[...]
        sgn = jnp.where(jax.lax.broadcasted_iota(jnp.int32, (P, P), 0) % 2 == 0, 1.0, -1.0).astype(f32)
        for jj in range(CR // P):
            j = lo // P + jj
            xh[p, 0, j] = _dot(fm, kvb[jj * P:(jj + 1) * P])
            H = _dot(fm, tie(hb[t, :, j * P:(j + 1) * P]), ((1,), (1,)))
            if j + 1 < NB:
                xh[p, 2, j + 1, :P] = sgn * H[:P]
                xh[p, 2, j + 1, P:] = sgn * H[P:]
            if j > 0:
                xh[p, 1, j, :P] = H[:P] - xh[p, 2, j, P:]
                xh[p, 1, j, P:] = H[P:] + xh[p, 2, j, :P]
            else:
                xh[p, 1, j] = H

    newdep = []

    def conv(p, c):
        for sl in range(c * 16 // NC, (c + 1) * 16 // NC):
            r0, r1 = slice(sl * 8, sl * 8 + 8), slice(P + sl * 8, P + sl * 8 + 8)
            for ib in range(0, NB, 4):
                acc = [None] * 4
                for j in range(ib + 4):
                    a, b = xh[p, 0, j, r0], xh[p, 0, j, r1]
                    for ii in range(4):
                        m = ib + ii - j
                        if m < 0:
                            continue
                        cc, d = xh[p, 1, m, r0], xh[p, 1, m, r1]
                        pr, pi = a * cc - b * d, a * d + b * cc
                        acc[ii] = [pr, pi] if acc[ii] is None else [acc[ii][0] + pr, acc[ii][1] + pi]
                for ii in range(4):
                    ys[p, ib + ii, r0] = acc[ii][0]
                    ys[p, ib + ii, r1] = acc[ii][1]
                yield ib

    def inv(t, p, c):
        gm = g_ref[...]
        for i in range(c * NB // NC, (c + 1) * NB // NC):
            r = slice(i * P, (i + 1) * P)
            y = _dot(gm, tie(ys[p, i].astype(bf16)))
            oa[t, r, :] = (qb[t, r, :].astype(f32) * (y + kvf[t % 3, r])).astype(bf16)

    def step(s, p, first=False, do_inv=True, last=False):
        if not last:
            for j in range(3):
                w_copy(s + 1, j).start()
            for n in range(3):
                a_copy(s + 1, n).start()
        a_copy(s, 3).start()
        for j in range(3):
            w_copy(s, j).wait()
        if do_inv:
            a_copy(s - 2, 3).wait()
        if not first:
            for n in range(3):
                a_copy(s, n).wait()
        for c in range(NC):
            if first and c * CR % XR == 0:
                x_copy(c * CR // XR).wait()
            @blk
            def _():
                b1(s, c, iter(()) if first else conv(1 - p, c))
                if first:
                    if c == 0:
                        for n in range(3):
                            a_copy(s, n).wait()
                else:
                    bpost(s - 1, c)
                fwd(s, p, c)
                if do_inv:
                    inv(s - 2, p, c)
        if first:
            wo_copy.wait()
        if do_inv:
            oa_copy(s - 2).start()

    step(0, 0, first=True, do_inv=False)
    step(1, 1, do_inv=False)
    if LOOP:
        def body(s, _):
            step(s, s % 2)
        jax.lax.fori_loop(2, NT - 1, body, None)
    else:
        for s in range(2, NT - 1):
            step(s, s % 2)
    step(NT - 1, 1, last=True)
    a_copy(NT - 2, 3).wait()
    a_copy(NT - 1, 3).wait()
    for c in range(NC):
        bpost(NT - 1, c)
    for i in range(8):
        r = slice(i * OR, (i + 1) * OR)
        @blk
        def _():
            rr = jnp.concatenate([rs[g, r, :] for g in range(NT)], axis=1)
            res = _dot(rr, jnp.concatenate([tie(kvw[g]) for g in range(NT)], axis=1)).astype(bf16)
            for g in range(NT):
                ob[g, r] = res[:, g * P:(g + 1) * P]
            ob_copy(i).start()
            h = 4
            if i < h:
                for c in range(i * NC // 4, (i + 1) * NC // 4):
                    list(conv(1, c))
                    inv(NT - 2, 0, c)
                if i == h - 1:
                    oa_copy(NT - 2).start()
            elif i < h + 2:
                for c in range((i - h) * NC // 2, (i - h + 1) * NC // 2):
                    inv(NT - 1, 1, c)
                if i == h + 1:
                    oa_copy(NT - 1).start()
    for t in range(NT):
        oa_copy(t).wait()
    for i in range(8):
        ob_copy(i).wait()


@jax.jit
def pallas_concat_heads__ssm_conv_h3__linear_attn_block__prompt_kernel(
    A_q, A_k, A_v, A_shift_k, A_ssm_k, A_ssm_D, B_x, B_wqkv, B_wo):
    hbm = pl.BlockSpec(memory_space=pl.ANY)
    vm = pl.BlockSpec(memory_space=pltpu.VMEM)
    V = pltpu.VMEM
    DMA = pltpu.SemaphoreType.DMA
    out = pl.pallas_call(
        _kernel,
        out_shape=jax.ShapeDtypeStruct((S, 2 * D), bf16),
        in_specs=[hbm, hbm, hbm, vm, hbm, vm, hbm, hbm, hbm, vm, vm, vm],
        out_specs=hbm, grid=(1,),
        scratch_shapes=[
            V((NT, S, P), bf16), V((NT, 3, D, P), bf16), V((D, D), bf16),
            V((NT, S, P), bf16), V((NT, S, P), bf16), V((NT, S, P), bf16), V((NT, P, S), bf16),
            V((NT, S, P), bf16), V((NT, D, P), bf16),
            V((2, 3, NB, 2 * P, P), f32), V((2, NB, 2 * P, P), f32), V((3, S, P), f32),
            V((NT, S, P), bf16), V((NT, S, P), bf16),
            V((NT, 8, P), f32), V((NT, P, P), f32), V((NT, 8, P), f32), pltpu.SMEM((1,), jnp.int32),
            DMA((4, NT)), DMA((NT, 3)), DMA(()), DMA((NT, 4)), DMA((NT,)), DMA((8, NT)),
        ],
        compiler_params=pltpu.CompilerParams(vmem_limit_bytes=100 * 1024 * 1024),
    )(A_q.reshape(S, D), A_k.reshape(S, D), A_v.reshape(S, D), A_shift_k.T, A_ssm_k, A_ssm_D,
      B_x.reshape(S, D), B_wqkv, B_wo, _F, _G, np.zeros((8, P), np.int32))
    return out.reshape(1, S, 2 * D)
```
